```python
import os as _os
_os.environ.setdefault("JAX_PLATFORMS", "cpu")
import jax
import jax.numpy as jnp

def _softmax(x, axis=-1):
    return jax.nn.softmax(x, axis=axis)
def _gelu(x):
    return jax.nn.gelu(x, approximate=True)
def _silu(x):
    return jax.nn.silu(x)
def _sigmoid(x):
    return jax.nn.sigmoid(x)
def _layernorm(x, axis=-1, eps=1e-5):
    m = jnp.mean(x, axis=axis, keepdims=True)
    v = jnp.var(x, axis=axis, keepdims=True)
    return (x - m) / jnp.sqrt(v + eps)
def _scatter_add(tgt, idx, src, axis=0):
    return tgt.at[idx].add(src)
def _segment_sum(src, seg, n):
    return jax.ops.segment_sum(src, seg, n)
class _Rng:
    def __init__(self, key):
        self._k = key
    def _next(self):
        self._k, sub = jax.random.split(self._k)
        return sub
    def normal(self, shape):
        return jax.random.normal(self._next(), shape, dtype=jnp.bfloat16)
    def randint(self, lo, hi, shape):
        return jax.random.randint(self._next(), shape, lo, hi, dtype=jnp.int32)
    def uniform(self, shape, lo=0.0, hi=1.0):
        return jax.random.uniform(self._next(), shape, jnp.bfloat16, lo, hi)
    def permutation(self, n):
        return jax.random.permutation(self._next(), n)


kernel_name = 'parallel_sum__sliding_block_cached__dense_activation_mish__decode'

def setup_inputs():
    _rng = _Rng(jax.random.key(int.from_bytes(__import__("os").urandom(4), "little")))
    _w = (lambda a: (lambda t: t.astype(jnp.bfloat16) if jnp.issubdtype(t.dtype, jnp.floating) else t)(jnp.asarray(a)))
    def _A_setup():
        B, Sq, D = 2, 1, 512
        Hq, Hkv, Sk, Dh = 32, 8, 32768, 128
        assert Hq % Hkv == 0, (Hq, Hkv)
        return {
            "x": _w((lambda *s: _rng.normal(s) * 0.05)(B, Sq, D)),
            "k_cache": _w((lambda *s: _rng.normal(s) * 0.8)(B, Hkv, Sk, Dh)),
            "v_cache": _w((lambda *s: _rng.normal(s) * 0.8)(B, Hkv, Sk, Dh)),
            "wq": _w((lambda *s: _rng.normal(s) * 0.8)(D, Hq * Dh) * (D ** -0.5)),
            "wo": _w((lambda *s: _rng.normal(s) * 0.8)(Hq * Dh, D) * ((Hq * Dh) ** -0.5)),
        }
    _A_in = _A_setup()

    def _B_setup():
        B, S, D, F = 2, 1, 512, 1792
        return {
            "x": _w((lambda *s: _rng.normal(s) * 0.05)(B, S, D)),
            "w1": _w((lambda *s: _rng.normal(s) * 0.4)(D, F) * (D ** -0.5)),
            "b1": _w((lambda *s: _rng.normal(s) * 0.05)(F)),
            "w2": _w((lambda *s: _rng.normal(s) * 0.05)(F, D) * (F ** -0.5)),
        }
    _B_in = _B_setup()

    return {
        "A_x": _A_in["x"],
        "A_k_cache": _A_in["k_cache"],
        "A_v_cache": _A_in["v_cache"],
        "A_wq": _A_in["wq"],
        "A_wo": _A_in["wo"],
        "B_x": _B_in["x"],
        "B_w1": _B_in["w1"],
        "B_b1": _B_in["b1"],
        "B_w2": _B_in["w2"],
    }

def reference(A_x, A_k_cache, A_v_cache, A_wq, A_wo, B_x, B_w1, B_b1, B_w2):
    def _A_ref(x, k_cache, v_cache, wq, wo):
        B, Sq, D = x.shape
        Hq, Dh = 32, 128
        Hkv, Sk = k_cache.shape[1], k_cache.shape[2]
        W = min(4096, max(256, Sk // 4))
        rep = Hq // Hkv
        q = (lambda x, *d: x.transpose(*d))((x @ wq).reshape(B, Sq, Hq, Dh), 0, 2, 1, 3)
        k = jnp.repeat(k_cache[:, :, Sk - W:, :], rep, axis=1)
        v = jnp.repeat(v_cache[:, :, Sk - W:, :], rep, axis=1)
        scores = jnp.einsum("bhqd,bhkd->bhqk", q, k) * (Dh ** -0.5)
        p = _softmax(scores, axis=-1)
        o = jnp.einsum("bhqk,bhkd->bhqd", p, v)
        return (lambda x, *d: x.transpose(*d))(o, 0, 2, 1, 3).reshape(B, Sq, Hq * Dh) @ wo

    def _B_ref(x, w1, b1, w2):
        h = jnp.einsum("bsd,df->bsf", x, w1) + b1
        sp = jnp.log1p(jnp.exp(-jnp.abs(h))) + jnp.where(h > 0, h, jnp.zeros_like(h))
        act = h * jnp.tanh(sp)
        return jnp.einsum("bsf,fd->bsd", act, w2)

    x = A_x
    xn = _layernorm(x, axis=-1)
    return x + _A_ref(xn, A_k_cache, A_v_cache, A_wq, A_wo) + _B_ref(xn, B_w1, B_b1, B_w2)
```

```python
import jax
import jax.numpy as jnp
from jax import lax
import jax.experimental.pallas as pl
import jax.experimental.pallas.tpu as pltpu

bf16, f32 = jnp.bfloat16, jnp.float32


@jax.jit
def pallas_parallel_sum__sliding_block_cached__dense_activation_mish__decode_kernel(
    A_x, A_k_cache, A_v_cache, A_wq, A_wo, B_x, B_w1, B_b1, B_w2,
):
    B, _, D = A_x.shape
    HQ, DH = 32, 128
    HKV, SK = A_k_cache.shape[1], A_k_cache.shape[2]
    W = min(4096, max(256, SK // 4))
    F = B_w1.shape[1]
    REP = HQ // HKV
    G = REP * DH
    w2_chunks = (896, 512, 256, 128)
    n2 = len(w2_chunks)

    def kernel(x_hbm, k_hbm, v_hbm, wq_hbm, wo_hbm, w1_hbm, b1_hbm, w2_hbm, o_ref,
               xb, b1b, kb, vb, wqb, wob, w1b, w2b, sem_h, sem_m):
        win = pl.ds(SK - W, W)

        def head_copies(h):
            col = pl.ds(pl.multiple_of(h * G, G), G)
            return (
                pltpu.make_async_copy(wq_hbm.at[:, col], wqb.at[h], sem_h.at[0, h]),
                pltpu.make_async_copy(k_hbm.at[:, h, win], kb.at[h], sem_h.at[1, h]),
                pltpu.make_async_copy(v_hbm.at[:, h, win], vb.at[h], sem_h.at[2, h]),
                pltpu.make_async_copy(wo_hbm.at[col, :], wob.at[h], sem_h.at[3, h]),
            )

        x_cp = pltpu.make_async_copy(x_hbm, xb, sem_m.at[0])
        b1_cp = pltpu.make_async_copy(b1_hbm, b1b, sem_m.at[1])
        w1_cp = pltpu.make_async_copy(w1_hbm, w1b, sem_m.at[2])
        w2_cps = []
        off = 0
        for i, n in enumerate(w2_chunks):
            w2_cps.append(pltpu.make_async_copy(w2_hbm.at[pl.ds(off, n)], w2b.at[pl.ds(off, n)], sem_m.at[3 + i]))
            off += n

        x_cp.start()
        for h in range(HKV):
            for c in head_copies(h):
                c.start()
        b1_cp.start()
        w1_cp.start()
        for c in w2_cps:
            c.start()

        row = lax.broadcasted_iota(jnp.int32, (8, DH), 0)
        x_cp.wait()
        x = xb[...].astype(f32)
        rowD = lax.broadcasted_iota(jnp.int32, (8, D), 0)
        x8 = jnp.where(rowD % 2 == 0, jnp.broadcast_to(x[0:1], (8, D)), jnp.broadcast_to(x[1:2], (8, D)))
        mean = jnp.mean(x8, axis=-1, keepdims=True)
        xc = x8 - mean
        var = jnp.mean(xc * xc, axis=-1, keepdims=True)
        xn = (xc / jnp.sqrt(var + 1e-5)).astype(bf16)

        def head(h, acc):
            wq_cp, k_cp, v_cp, wo_cp = head_copies(h)
            wq_cp.wait()
            qq = jnp.dot(xn, wqb[h], preferred_element_type=f32)
            q = qq[:, 0:DH]
            for j in range(1, REP):
                q = jnp.where(row // 2 == j, qq[:, j * DH:(j + 1) * DH], q)
            q = q.astype(bf16)
            k_cp.wait()
            nt = (((1,), (1,)), ((), ()))
            s0 = lax.dot_general(q, kb[h, 0], nt, preferred_element_type=f32)
            s1 = lax.dot_general(q, kb[h, 1], nt, preferred_element_type=f32)
            rowW = lax.broadcasted_iota(jnp.int32, (8, W), 0)
            s = jnp.where(rowW % 2 == 0, s0, s1) * (DH ** -0.5)
            m = jnp.max(s, axis=-1, keepdims=True)
            p = jnp.exp(s - m)
            l = jnp.sum(p, axis=-1, keepdims=True)
            p = p.astype(bf16)
            v_cp.wait()
            o0 = jnp.dot(p, vb[h, 0], preferred_element_type=f32)
            o1 = jnp.dot(p, vb[h, 1], preferred_element_type=f32)
            o = jnp.where(row % 2 == 0, o0, o1) / l
            lhs = jnp.concatenate([jnp.where(row // 2 == j, o, 0.0) for j in range(REP)], axis=-1).astype(bf16)
            wo_cp.wait()
            return acc + jnp.dot(lhs, wob[h], preferred_element_type=f32)

        acc = lax.fori_loop(0, HKV, head, jnp.zeros((8, D), f32))
        acc = acc + pltpu.roll(acc, 4, 0)
        acc = acc + pltpu.roll(acc, 2, 0)
        acc = acc + x8

        b1_cp.wait()
        w1_cp.wait()
        hh = jnp.dot(xn, w1b[...], preferred_element_type=f32)
        b1 = b1b[...].astype(f32)
        hh = hh + jnp.concatenate([jnp.broadcast_to(b1[i:i + 1], (8, 128)) for i in range(F // 128)], axis=-1)
        sp = jnp.log1p(jnp.exp(-jnp.abs(hh))) + jnp.where(hh > 0, hh, 0.0)
        act = (hh * jnp.tanh(sp)).astype(bf16)
        off = 0
        for c, n in zip(w2_cps, w2_chunks):
            c.wait()
            acc = acc + jnp.dot(act[:, off:off + n], w2b[pl.ds(off, n), :], preferred_element_type=f32)
            off += n
        o_ref[...] = acc[0:2].astype(o_ref.dtype)

    anyspec = pl.BlockSpec(memory_space=pl.ANY)
    out = pl.pallas_call(
        kernel,
        out_shape=jax.ShapeDtypeStruct((B, D), bf16),
        in_specs=[anyspec] * 8,
        out_specs=pl.BlockSpec(memory_space=pltpu.VMEM),
        scratch_shapes=[
            pltpu.VMEM((B, D), bf16),
            pltpu.VMEM((F // 128, 128), bf16),
            pltpu.VMEM((HKV, B, W, DH), bf16),
            pltpu.VMEM((HKV, B, W, DH), bf16),
            pltpu.VMEM((HKV, D, G), bf16),
            pltpu.VMEM((HKV, G, D), bf16),
            pltpu.VMEM((D, F), bf16),
            pltpu.VMEM((F, D), bf16),
            pltpu.SemaphoreType.DMA((4, HKV)),
            pltpu.SemaphoreType.DMA((3 + n2,)),
        ],
        compiler_params=pltpu.CompilerParams(vmem_limit_bytes=64 * 1024 * 1024),
    )(A_x.reshape(B, D), A_k_cache, A_v_cache, A_wq, A_wo, B_w1, B_b1.reshape(F // 128, 128), B_w2)
    return out.reshape(B, 1, D)
```

```python
import functools, contextlib
import jax, jax.numpy as jnp
from jax import lax
import jax.experimental.pallas as pl
import jax.experimental.pallas.tpu as pltpu

B, D, HQ, HKV, SK, DH, F = 2, 512, 32, 8, 32768, 128, 1792
W = 4096
REP = HQ // HKV
G = REP * DH
bf16, f32 = jnp.bfloat16, jnp.float32

def make(scopes=False, nobounds=True, nosem=True, CH=512, KR=128, w2_tail=(512, 256, 128)):
    sc = (lambda n: jax.named_scope(n)) if scopes else (lambda n: contextlib.nullcontext())
    NC = W // CH
    PP = CH // KR
    WR = KR * DH // D
    S_Q, S_K, S_V, S_O, S_X, S_W1, S_W2 = 0, 1, 2, 3, 4, 5, 6
    n_t = len(w2_tail)
    assert sum(w2_tail) == F // 2
    assert (F // 2) % (WR * PP) == 0 and all(n % WR == 0 for n in w2_tail)

    def kernel(x_hbm, k_hbm, v_hbm, wq_hbm, wo_hbm, w1_hbm, b1_hbm, w2_hbm, o_ref,
               xb, b1b, kb, vb, wqb, wob, w1b, w2b, s_scr, sems):

        def start(src, dst, sem, prio):
            pltpu.make_async_copy(src, dst, sems.at[sem]).start(priority=prio)

        def wait(buf, sem):
            pltpu.make_async_copy(buf, buf, sems.at[sem]).wait()

        def issue_kv(hbm, buf, sem, h, c):
            for u in range(PP):
                r = pl.multiple_of(c * CH + u * KR, KR)
                for b in (1, 0):
                    start(hbm.at[b, h, pl.ds(SK - W + r, KR)], buf.at[h, b, pl.ds(r, KR)], sem, b)

        def issue_wq(h, i0, n):
            col = pl.ds(pl.multiple_of(h * G, G), G)
            for i in range(i0, i0 + n):
                for half in (1, 0):
                    r = pl.ds(half * (D // 2) + i * WR, WR)
                    start(wq_hbm.at[r, col], wqb.at[h, r], S_Q, half)

        def issue_wo(h, i0, n):
            for i in range(i0, i0 + n):
                for half in (1, 0):
                    r = half * (G // 2) + i * WR
                    start(wo_hbm.at[pl.ds(pl.multiple_of(h * G + r, WR), WR)], wob.at[h, pl.ds(r, WR)], S_O, half)

        def issue_w2(c):
            for u in range(PP):
                i = c * PP + u
                r = pl.multiple_of(i * WR, WR)
                sem1 = S_W2 + 1
                off = 0
                for n in w2_tail[:-1]:
                    off += n
                    sem1 = sem1 + (r >= off).astype(jnp.int32)
                start(w2_hbm.at[pl.ds(F // 2 + r, WR)], w2b.at[pl.ds(F // 2 + r, WR)], sem1, 1)
                start(w2_hbm.at[pl.ds(r, WR)], w2b.at[pl.ds(r, WR)], S_W2, 0)

        NW = D // 2 // WR
        with sc("prologue_issue"):
            start(x_hbm, xb, S_X, 0)
            start(b1_hbm, b1b, S_W1, 0)

            def w1_body(i, _):
                for half in (1, 0):
                    r = pl.ds(pl.multiple_of(half * (D // 2) + i * 8, 8), 8)
                    start(w1_hbm.at[r], w1b.at[r], S_W1, half)
            lax.fori_loop(0, D // 16, w1_body, None, unroll=2)
            issue_wq(0, 0, NW)
            lax.fori_loop(0, NC, lambda c, _: issue_kv(k_hbm, kb, S_K, 0, c), None)

        row = lax.broadcasted_iota(jnp.int32, (8, DH), 0)
        with sc("ln_mlp1"):
            wait(xb, S_X)
            x = xb[...].astype(f32)
            rowD = lax.broadcasted_iota(jnp.int32, (8, D), 0)
            x8 = jnp.where(rowD % 2 == 0, jnp.broadcast_to(x[0:1], (8, D)), jnp.broadcast_to(x[1:2], (8, D)))
            mean = jnp.mean(x8, axis=-1, keepdims=True)
            xc = x8 - mean
            var = jnp.mean(xc * xc, axis=-1, keepdims=True)
            xn = (xc / jnp.sqrt(var + 1e-5)).astype(bf16)
            wait(b1b, S_W1)
            wait(w1b, S_W1)
            hh = jnp.dot(xn, w1b[...], preferred_element_type=f32)
            b1 = b1b[...].astype(f32)
            hh = hh + jnp.concatenate([jnp.broadcast_to(b1[i:i + 1], (8, 128)) for i in range(F // 128)], axis=-1)
            sp = jnp.log1p(jnp.exp(-jnp.abs(hh))) + jnp.where(hh > 0, hh, 0.0)
            act = (hh * jnp.tanh(sp)).astype(bf16)

        with sc("prologue_issue2"):
            lax.fori_loop(0, NC, lambda c, _: issue_kv(v_hbm, vb, S_V, 0, c), None)
            issue_wo(0, 0, NW)

        nt = (((1,), (1,)), ((), ()))
        n_w2_steps = F // 2 // WR // PP

        def head(h, acc):
            more = h < HKV - 1
            with sc("q"):
                wait(wqb.at[h], S_Q)
                qq = jnp.zeros((8, G), f32)
                for u in range(2):
                    pl.when(more)(lambda: issue_wq(h + 1, u * NW // 2, NW // 2))
                    ks = slice(u * D // 2, (u + 1) * D // 2)
                    qq = qq + jnp.dot(xn[:, ks], wqb[h, ks, :], preferred_element_type=f32)
                q = qq[:, 0:DH]
                for j in range(1, REP):
                    q = jnp.where(row // 2 == j, qq[:, j * DH:(j + 1) * DH], q)
                q = q.astype(bf16)

            with sc("qk"):
                wait(kb.at[h], S_K)

                def s_step(c, mrun):
                    pl.when(more)(lambda: issue_kv(k_hbm, kb, S_K, h + 1, c))
                    pl.when(jnp.logical_and(jnp.logical_not(more), c < n_w2_steps))(lambda: issue_w2(c))
                    r = pl.ds(pl.multiple_of(c * CH, CH), CH)
                    s0 = lax.dot_general(q, kb[h, 0, r, :], nt, preferred_element_type=f32)
                    s1 = lax.dot_general(q, kb[h, 1, r, :], nt, preferred_element_type=f32)
                    rowC = lax.broadcasted_iota(jnp.int32, (8, CH), 0)
                    s = jnp.where(rowC % 2 == 0, s0, s1) * (DH ** -0.5)
                    s_scr[c] = s
                    for t in range(CH // 128):
                        mrun = jnp.maximum(mrun, s[:, t * 128:(t + 1) * 128])
                    return mrun
                mrun = lax.fori_loop(0, NC, s_step, jnp.full((8, 128), -jnp.inf, f32))
                m = jnp.max(mrun, axis=-1, keepdims=True)

            with sc("pv"):
                wait(vb.at[h], S_V)

                def pv_step(c, carry):
                    lrun, o0, o1 = carry
                    pl.when(more)(lambda: issue_kv(v_hbm, vb, S_V, h + 1, c))
                    r = pl.ds(pl.multiple_of(c * CH, CH), CH)
                    p = jnp.exp(s_scr[c] - m)
                    for t in range(CH // 128):
                        lrun = lrun + p[:, t * 128:(t + 1) * 128]
                    p = p.astype(bf16)
                    o0 = o0 + jnp.dot(p, vb[h, 0, r, :], preferred_element_type=f32)
                    o1 = o1 + jnp.dot(p, vb[h, 1, r, :], preferred_element_type=f32)
                    return lrun, o0, o1
                z = jnp.zeros((8, DH), f32)
                lrun, o0, o1 = lax.fori_loop(0, NC, pv_step, (z, z, z))
                o = jnp.where(row % 2 == 0, o0, o1) / jnp.sum(lrun, axis=-1, keepdims=True)
                lhs = jnp.concatenate([jnp.where(row // 2 == j, o, 0.0) for j in range(REP)], axis=-1).astype(bf16)

            with sc("wo"):
                wait(wob.at[h], S_O)
                for u in range(2):
                    pl.when(more)(lambda: issue_wo(h + 1, u * NW // 2, NW // 2))
                    ks = slice(u * G // 2, (u + 1) * G // 2)
                    acc = acc + jnp.dot(lhs[:, ks], wob[h, ks, :], preferred_element_type=f32)
            return acc

        acc = lax.fori_loop(0, HKV, head, jnp.zeros((8, D), f32))
        acc = acc + pltpu.roll(acc, 4, 0)
        acc = acc + pltpu.roll(acc, 2, 0)
        acc = acc + x8

        off = 0
        for i, n in enumerate((F // 2,) + tuple(w2_tail)):
            with sc(f"wait_w2_{i}"):
                wait(w2b.at[pl.ds(off, n)], S_W2 + i)
            with sc(f"w2_{i}"):
                acc = acc + jnp.dot(act[:, off:off + n], w2b[pl.ds(off, n), :], preferred_element_type=f32)
            off += n
        o_ref[...] = acc[0:2].astype(o_ref.dtype)

    def fn(A_x, A_k, A_v, A_wq, A_wo, B_x, B_w1, B_b1, B_w2):
        anyspec = pl.BlockSpec(memory_space=pl.ANY)
        out = pl.pallas_call(
            kernel,
            out_shape=jax.ShapeDtypeStruct((B, D), bf16),
            in_specs=[anyspec] * 8,
            out_specs=pl.BlockSpec(memory_space=pltpu.VMEM),
            scratch_shapes=[
                pltpu.VMEM((B, D), bf16),
                pltpu.VMEM((F // 128, 128), bf16),
                pltpu.VMEM((HKV, B, W, DH), bf16),
                pltpu.VMEM((HKV, B, W, DH), bf16),
                pltpu.VMEM((HKV, D, G), bf16),
                pltpu.VMEM((HKV, G, D), bf16),
                pltpu.VMEM((D, F), bf16),
                pltpu.VMEM((F, D), bf16),
                pltpu.VMEM((NC, 8, CH), f32),
                pltpu.SemaphoreType.DMA((S_W2 + 1 + n_t,)),
            ],
            compiler_params=pltpu.CompilerParams(vmem_limit_bytes=64 * 1024 * 1024,
                                                 disable_bounds_checks=nobounds, disable_semaphore_checks=nosem),
        )(A_x.reshape(B, D), A_k, A_v, A_wq, A_wo, B_w1, B_b1.reshape(F // 128, 128), B_w2)
        return out.reshape(B, 1, D)
    return fn


@jax.jit
def pallas_parallel_sum__sliding_block_cached__dense_activation_mish__decode_kernel(
        A_x, A_k_cache, A_v_cache, A_wq, A_wo, B_x, B_w1, B_b1, B_w2):
    return make()(A_x, A_k_cache, A_v_cache, A_wq, A_wo, B_x, B_w1, B_b1, B_w2)
```

```python
import jax
import jax.numpy as jnp
from jax import lax
import jax.experimental.pallas as pl
import jax.experimental.pallas.tpu as pltpu

_HQ, _DH = 32, 128
_ROWS = 8
_KV_PIECE = 128
_PAIRS_PER_STEP = 4
_W2_TAIL = (512, 256, 128)

_S_K, _S_V, _S_WO, _S_X, _S_B1, _S_W1, _S_WQ, _S_W2 = range(8)


def _kernel(x_hbm, k_hbm, v_hbm, wq_hbm, wo_hbm, w1_hbm, b1_hbm, w2_hbm, o_ref,
            x_buf, b1_buf, k_buf, v_buf, wq_buf, wo_buf, w1_buf, w2_buf, sems):
  f32, bf16 = jnp.float32, jnp.bfloat16
  hkv, _, win, dh = k_buf.shape
  sk = k_hbm.shape[2]
  d, f = w1_buf.shape
  rep = _HQ // hkv
  g = rep * dh
  w_piece = _KV_PIECE * dh // d

  def start(src, dst, sem, thread):
    pltpu.make_async_copy(src, dst, sems.at[sem]).start(priority=thread)

  def wait(buf, sem):
    pltpu.make_async_copy(buf, buf, sems.at[sem]).wait()

  def fetch_window(hbm, buf, sem, h):
    def step(i, _):
      for u in range(_PAIRS_PER_STEP):
        r = pl.multiple_of((i * _PAIRS_PER_STEP + u) * _KV_PIECE, _KV_PIECE)
        for b in (1, 0):
          start(hbm.at[b, h, pl.ds(sk - win + r, _KV_PIECE)],
                buf.at[h, b, pl.ds(r, _KV_PIECE)], sem, b)
    lax.fori_loop(0, win // (_KV_PIECE * _PAIRS_PER_STEP), step, None)

  def fetch_wide(hbm, buf, sem, col_pieces):
    n = hbm.shape[1] // col_pieces
    def step(i, _):
      for c in range(col_pieces):
        for half in (1, 0):
          r = pl.ds(pl.multiple_of(half * (d // 2) + i * 8, 8), 8)
          start(hbm.at[r, pl.ds(c * n, n)], buf.at[r, pl.ds(c * n, n)], sem, half)
    lax.fori_loop(0, d // 16, step, None, unroll=2)

  def fetch_wo(h):
    for i in range(g // 2 // w_piece):
      for half in (1, 0):
        r = half * (g // 2) + i * w_piece
        start(wo_hbm.at[pl.ds(pl.multiple_of(h * g + r, w_piece), w_piece)],
              wo_buf.at[h, pl.ds(r, w_piece)], _S_WO, half)

  def fetch_w2():
    def step(i, _):
      for u in range(_PAIRS_PER_STEP):
        r = pl.multiple_of((i * _PAIRS_PER_STEP + u) * w_piece, w_piece)
        sem, end = _S_W2 + 1, 0
        for n in _W2_TAIL[:-1]:
          end += n
          sem = sem + (r >= end).astype(jnp.int32)
        start(w2_hbm.at[pl.ds(f // 2 + r, w_piece)],
              w2_buf.at[pl.ds(f // 2 + r, w_piece)], sem, 1)
        start(w2_hbm.at[pl.ds(r, w_piece)], w2_buf.at[pl.ds(r, w_piece)], _S_W2, 0)
    lax.fori_loop(0, f // 2 // (w_piece * _PAIRS_PER_STEP), step, None)

  def row_iota(n):
    return lax.broadcasted_iota(jnp.int32, (_ROWS, n), 0)

  start(x_hbm, x_buf, _S_X, 0)
  start(b1_hbm, b1_buf, _S_B1, 0)
  fetch_wide(w1_hbm, w1_buf, _S_W1, 1)
  fetch_wide(wq_hbm, wq_buf, _S_WQ, 2)

  wait(x_buf, _S_X)
  x = x_buf[...].astype(f32)
  x = jnp.where(row_iota(d) % 2 == 0, jnp.broadcast_to(x[0:1], (_ROWS, d)),
                jnp.broadcast_to(x[1:2], (_ROWS, d)))
  xc = x - jnp.mean(x, axis=-1, keepdims=True)
  var = jnp.mean(xc * xc, axis=-1, keepdims=True)
  xn = (xc / jnp.sqrt(var + 1e-5)).astype(bf16)

  wait(b1_buf, _S_B1)
  wait(w1_buf, _S_W1)
  b1 = b1_buf[...].astype(f32)
  hid = jnp.dot(xn, w1_buf[...], preferred_element_type=f32) + jnp.concatenate(
      [jnp.broadcast_to(b1[i:i + 1], (_ROWS, 128)) for i in range(f // 128)], axis=-1)
  softplus = jnp.log1p(jnp.exp(-jnp.abs(hid))) + jnp.where(hid > 0, hid, 0.0)
  act = (hid * jnp.tanh(softplus)).astype(bf16)

  fetch_window(k_hbm, k_buf, _S_K, 0)
  fetch_window(v_hbm, v_buf, _S_V, 0)
  fetch_wo(0)
  wait(wq_buf, _S_WQ)

  def kv_head(h, acc):
    more = h < hkv - 1
    row = row_iota(dh)

    q_all = jnp.dot(xn, wq_buf[:, pl.ds(pl.multiple_of(h * g, g), g)],
                    preferred_element_type=f32)
    q = q_all[:, :dh]
    for j in range(1, rep):
      q = jnp.where(row // 2 == j, q_all[:, j * dh:(j + 1) * dh], q)
    q = q.astype(bf16)

    wait(k_buf.at[h], _S_K)
    pl.when(more)(lambda: fetch_window(k_hbm, k_buf, _S_K, h + 1))
    pl.when(jnp.logical_not(more))(fetch_w2)
    s0, s1 = (lax.dot_general(q, k_buf[h, b], (((1,), (1,)), ((), ())),
                              preferred_element_type=f32) for b in range(2))
    s = jnp.where(row_iota(win) % 2 == 0, s0, s1) * (dh ** -0.5)
    p = jnp.exp(s - jnp.max(s, axis=-1, keepdims=True))
    denom = jnp.sum(p, axis=-1, keepdims=True)
    p = p.astype(bf16)

    wait(v_buf.at[h], _S_V)
    pl.when(more)(lambda: fetch_window(v_hbm, v_buf, _S_V, h + 1))
    o0, o1 = (jnp.dot(p, v_buf[h, b], preferred_element_type=f32) for b in range(2))
    o = jnp.where(row % 2 == 0, o0, o1) / denom
    o = jnp.concatenate([jnp.where(row // 2 == j, o, 0.0) for j in range(rep)],
                        axis=-1).astype(bf16)

    wait(wo_buf.at[h], _S_WO)
    pl.when(more)(lambda: fetch_wo(h + 1))
    return acc + jnp.dot(o, wo_buf[h], preferred_element_type=f32)

  acc = lax.fori_loop(0, hkv, kv_head, jnp.zeros((_ROWS, d), f32))
  acc = acc + pltpu.roll(acc, 4, 0)
  acc = acc + pltpu.roll(acc, 2, 0)
  acc = acc + x

  lo = 0
  for i, n in enumerate((f // 2,) + _W2_TAIL):
    wait(w2_buf.at[pl.ds(lo, n)], _S_W2 + i)
    acc = acc + jnp.dot(act[:, lo:lo + n], w2_buf[pl.ds(lo, n), :],
                        preferred_element_type=f32)
    lo += n
  o_ref[...] = acc[0:2].astype(o_ref.dtype)


@jax.jit
def pallas_parallel_sum__sliding_block_cached__dense_activation_mish__decode_kernel(
    A_x: jax.Array,
    A_k_cache: jax.Array,
    A_v_cache: jax.Array,
    A_wq: jax.Array,
    A_wo: jax.Array,
    B_x: jax.Array,
    B_w1: jax.Array,
    B_b1: jax.Array,
    B_w2: jax.Array,
):
  del B_x
  b, sq, d = A_x.shape
  hkv, sk, dh = A_k_cache.shape[1:]
  f = B_w1.shape[1]
  win = min(4096, max(256, sk // 4))
  g = _HQ // hkv * dh
  w_piece = _KV_PIECE * dh // d
  assert (b, sq, dh) == (2, 1, _DH) and _HQ // hkv * b == _ROWS
  assert win % (_KV_PIECE * _PAIRS_PER_STEP) == 0 and d % 32 == 0 and f % 128 == 0
  assert g % (2 * w_piece) == 0 and (f // 2) % (w_piece * _PAIRS_PER_STEP) == 0
  assert sum(_W2_TAIL) == f // 2 and all(n % w_piece == 0 for n in _W2_TAIL)

  dtype = A_x.dtype
  out = pl.pallas_call(
      _kernel,
      out_shape=jax.ShapeDtypeStruct((b, d), dtype),
      in_specs=[pl.BlockSpec(memory_space=pl.ANY)] * 8,
      out_specs=pl.BlockSpec(memory_space=pltpu.VMEM),
      scratch_shapes=[
          pltpu.VMEM((b, d), dtype),
          pltpu.VMEM((f // 128, 128), dtype),
          pltpu.VMEM((hkv, b, win, dh), dtype),
          pltpu.VMEM((hkv, b, win, dh), dtype),
          pltpu.VMEM(A_wq.shape, dtype),
          pltpu.VMEM((hkv, g, d), dtype),
          pltpu.VMEM(B_w1.shape, dtype),
          pltpu.VMEM(B_w2.shape, dtype),
          pltpu.SemaphoreType.DMA((_S_W2 + 1 + len(_W2_TAIL),)),
      ],
      compiler_params=pltpu.CompilerParams(
          vmem_limit_bytes=64 * 1024 * 1024,
          disable_semaphore_checks=True,
      ),
  )(A_x.reshape(b, d), A_k_cache, A_v_cache, A_wq, A_wo, B_w1,
    B_b1.reshape(f // 128, 128), B_w2)
  return out.reshape(b, sq, d)
```

```python
import jax
import jax.numpy as jnp
from jax import lax
import jax.experimental.pallas as pl
import jax.experimental.pallas.tpu as pltpu

_HQ, _DH = 32, 128
_ROWS = 8
_KV_PIECE = 64
_PAIRS_PER_STEP = 4
_W2_TAIL = (512, 256, 128)

_S_K, _S_V, _S_WO, _S_X, _S_B1, _S_W1, _S_WQ, _S_W2 = range(8)


def _kernel(x_hbm, k_hbm, v_hbm, wq_hbm, wo_hbm, w1_hbm, b1_hbm, w2_hbm, o_ref,
            x_buf, b1_buf, k_buf, v_buf, wq_buf, wo_buf, w1_buf, w2_buf, sems):
  f32, bf16 = jnp.float32, jnp.bfloat16
  hkv, _, win, dh = k_buf.shape
  sk = k_hbm.shape[2]
  d, f = w1_buf.shape
  rep = _HQ // hkv
  g = rep * dh
  w_piece = _KV_PIECE * dh // d

  def start(src, dst, sem, thread):
    pltpu.make_async_copy(src, dst, sems.at[sem]).start(priority=thread)

  def wait(buf, sem):
    pltpu.make_async_copy(buf, buf, sems.at[sem]).wait()

  def fetch_window(hbm, buf, sem, h):
    def step(i, _):
      for u in range(_PAIRS_PER_STEP):
        r = pl.multiple_of((i * _PAIRS_PER_STEP + u) * _KV_PIECE, _KV_PIECE)
        for b in (1, 0):
          start(hbm.at[b, h, pl.ds(sk - win + r, _KV_PIECE)],
                buf.at[h, b, pl.ds(r, _KV_PIECE)], sem, b)
    lax.fori_loop(0, win // (_KV_PIECE * _PAIRS_PER_STEP), step, None)

  def fetch_wide(hbm, buf, sem):
    col_pieces = pl.cdiv(8 * hbm.shape[1], _KV_PIECE * dh)
    n = hbm.shape[1] // col_pieces
    assert n * col_pieces == hbm.shape[1] and n % 128 == 0
    def step(i, _):
      for c in range(col_pieces):
        for half in (1, 0):
          r = pl.ds(pl.multiple_of(half * (d // 2) + i * 8, 8), 8)
          start(hbm.at[r, pl.ds(c * n, n)], buf.at[r, pl.ds(c * n, n)], sem, half)
    lax.fori_loop(0, d // 16, step, None, unroll=2)

  def fetch_wo(h):
    for i in range(g // 2 // w_piece):
      for half in (1, 0):
        r = half * (g // 2) + i * w_piece
        start(wo_hbm.at[pl.ds(pl.multiple_of(h * g + r, w_piece), w_piece)],
              wo_buf.at[h, pl.ds(r, w_piece)], _S_WO, half)

  def fetch_w2():
    def step(i, _):
      for u in range(_PAIRS_PER_STEP):
        r = pl.multiple_of((i * _PAIRS_PER_STEP + u) * w_piece, w_piece)
        sem, end = _S_W2 + 1, 0
        for n in _W2_TAIL[:-1]:
          end += n
          sem = sem + (r >= end).astype(jnp.int32)
        start(w2_hbm.at[pl.ds(f // 2 + r, w_piece)],
              w2_buf.at[pl.ds(f // 2 + r, w_piece)], sem, 1)
        start(w2_hbm.at[pl.ds(r, w_piece)], w2_buf.at[pl.ds(r, w_piece)], _S_W2, 0)
    lax.fori_loop(0, f // 2 // (w_piece * _PAIRS_PER_STEP), step, None)

  def row_iota(n):
    return lax.broadcasted_iota(jnp.int32, (_ROWS, n), 0)

  start(x_hbm, x_buf, _S_X, 0)
  start(b1_hbm, b1_buf, _S_B1, 0)
  fetch_wide(w1_hbm, w1_buf, _S_W1)
  fetch_wide(wq_hbm, wq_buf, _S_WQ)

  wait(x_buf, _S_X)
  x = x_buf[...].astype(f32)
  x = jnp.where(row_iota(d) % 2 == 0, jnp.broadcast_to(x[0:1], (_ROWS, d)),
                jnp.broadcast_to(x[1:2], (_ROWS, d)))
  xc = x - jnp.mean(x, axis=-1, keepdims=True)
  var = jnp.mean(xc * xc, axis=-1, keepdims=True)
  xn = (xc / jnp.sqrt(var + 1e-5)).astype(bf16)

  wait(b1_buf, _S_B1)
  wait(w1_buf, _S_W1)
  b1 = b1_buf[...].astype(f32)
  hid = jnp.dot(xn, w1_buf[...], preferred_element_type=f32) + jnp.concatenate(
      [jnp.broadcast_to(b1[i:i + 1], (_ROWS, 128)) for i in range(f // 128)], axis=-1)
  softplus = jnp.log1p(jnp.exp(-jnp.abs(hid))) + jnp.where(hid > 0, hid, 0.0)
  act = (hid * jnp.tanh(softplus)).astype(bf16)

  fetch_window(k_hbm, k_buf, _S_K, 0)
  fetch_window(v_hbm, v_buf, _S_V, 0)
  fetch_wo(0)
  wait(wq_buf, _S_WQ)

  def kv_head(h, acc):
    more = h < hkv - 1
    row = row_iota(dh)

    q_all = jnp.dot(xn, wq_buf[:, pl.ds(pl.multiple_of(h * g, g), g)],
                    preferred_element_type=f32)
    q = q_all[:, :dh]
    for j in range(1, rep):
      q = jnp.where(row // 2 == j, q_all[:, j * dh:(j + 1) * dh], q)
    q = q.astype(bf16)

    wait(k_buf.at[h], _S_K)
    pl.when(more)(lambda: fetch_window(k_hbm, k_buf, _S_K, h + 1))
    pl.when(jnp.logical_not(more))(fetch_w2)
    s0, s1 = (lax.dot_general(q, k_buf[h, b], (((1,), (1,)), ((), ())),
                              preferred_element_type=f32) for b in range(2))
    s = jnp.where(row_iota(win) % 2 == 0, s0, s1) * (dh ** -0.5)
    p = jnp.exp(s - jnp.max(s, axis=-1, keepdims=True))
    denom = jnp.sum(p, axis=-1, keepdims=True)
    p = p.astype(bf16)

    wait(v_buf.at[h], _S_V)
    pl.when(more)(lambda: fetch_window(v_hbm, v_buf, _S_V, h + 1))
    o0, o1 = (jnp.dot(p, v_buf[h, b], preferred_element_type=f32) for b in range(2))
    o = jnp.where(row % 2 == 0, o0, o1) / denom
    o = jnp.concatenate([jnp.where(row // 2 == j, o, 0.0) for j in range(rep)],
                        axis=-1).astype(bf16)

    wait(wo_buf.at[h], _S_WO)
    pl.when(more)(lambda: fetch_wo(h + 1))
    return acc + jnp.dot(o, wo_buf[h], preferred_element_type=f32)

  acc = lax.fori_loop(0, hkv, kv_head, jnp.zeros((_ROWS, d), f32))
  acc = acc + pltpu.roll(acc, 4, 0)
  acc = acc + pltpu.roll(acc, 2, 0)
  acc = acc + x

  lo = 0
  for i, n in enumerate((f // 2,) + _W2_TAIL):
    wait(w2_buf.at[pl.ds(lo, n)], _S_W2 + i)
    acc = acc + jnp.dot(act[:, lo:lo + n], w2_buf[pl.ds(lo, n), :],
                        preferred_element_type=f32)
    lo += n
  o_ref[...] = acc[0:2].astype(o_ref.dtype)


@jax.jit
def pallas_parallel_sum__sliding_block_cached__dense_activation_mish__decode_kernel(
    A_x: jax.Array,
    A_k_cache: jax.Array,
    A_v_cache: jax.Array,
    A_wq: jax.Array,
    A_wo: jax.Array,
    B_x: jax.Array,
    B_w1: jax.Array,
    B_b1: jax.Array,
    B_w2: jax.Array,
):
  del B_x
  b, sq, d = A_x.shape
  hkv, sk, dh = A_k_cache.shape[1:]
  f = B_w1.shape[1]
  win = min(4096, max(256, sk // 4))
  g = _HQ // hkv * dh
  w_piece = _KV_PIECE * dh // d
  assert (b, sq, dh) == (2, 1, _DH) and _HQ // hkv * b == _ROWS
  assert win % (_KV_PIECE * _PAIRS_PER_STEP) == 0 and d % 32 == 0 and f % 128 == 0
  assert g % (2 * w_piece) == 0 and (f // 2) % (w_piece * _PAIRS_PER_STEP) == 0
  assert sum(_W2_TAIL) == f // 2 and all(n % w_piece == 0 for n in _W2_TAIL)

  dtype = A_x.dtype
  out = pl.pallas_call(
      _kernel,
      out_shape=jax.ShapeDtypeStruct((b, d), dtype),
      in_specs=[pl.BlockSpec(memory_space=pl.ANY)] * 8,
      out_specs=pl.BlockSpec(memory_space=pltpu.VMEM),
      scratch_shapes=[
          pltpu.VMEM((b, d), dtype),
          pltpu.VMEM((f // 128, 128), dtype),
          pltpu.VMEM((hkv, b, win, dh), dtype),
          pltpu.VMEM((hkv, b, win, dh), dtype),
          pltpu.VMEM(A_wq.shape, dtype),
          pltpu.VMEM((hkv, g, d), dtype),
          pltpu.VMEM(B_w1.shape, dtype),
          pltpu.VMEM(B_w2.shape, dtype),
          pltpu.SemaphoreType.DMA((_S_W2 + 1 + len(_W2_TAIL),)),
      ],
      compiler_params=pltpu.CompilerParams(
          vmem_limit_bytes=64 * 1024 * 1024,
          disable_semaphore_checks=True,
      ),
  )(A_x.reshape(b, d), A_k_cache, A_v_cache, A_wq, A_wo, B_w1,
    B_b1.reshape(f // 128, 128), B_w2)
  return out.reshape(b, sq, d)
```
